```python
import os as _os
_os.environ.setdefault("JAX_PLATFORMS", "cpu")
import jax
import jax.numpy as jnp

def _softmax(x, axis=-1):
    return jax.nn.softmax(x, axis=axis)
def _gelu(x):
    return jax.nn.gelu(x, approximate=True)
def _silu(x):
    return jax.nn.silu(x)
def _sigmoid(x):
    return jax.nn.sigmoid(x)
def _layernorm(x, axis=-1, eps=1e-5):
    m = jnp.mean(x, axis=axis, keepdims=True)
    v = jnp.var(x, axis=axis, keepdims=True)
    return (x - m) / jnp.sqrt(v + eps)
def _scatter_add(tgt, idx, src, axis=0):
    return tgt.at[idx].add(src)
def _segment_sum(src, seg, n):
    return jax.ops.segment_sum(src, seg, n)
class _Rng:
    def __init__(self, key):
        self._k = key
    def _next(self):
        self._k, sub = jax.random.split(self._k)
        return sub
    def normal(self, shape):
        return jax.random.normal(self._next(), shape, dtype=jnp.bfloat16)
    def randint(self, lo, hi, shape):
        return jax.random.randint(self._next(), shape, lo, hi, dtype=jnp.int32)
    def uniform(self, shape, lo=0.0, hi=1.0):
        return jax.random.uniform(self._next(), shape, jnp.bfloat16, lo, hi)
    def permutation(self, n):
        return jax.random.permutation(self._next(), n)


kernel_name = 'sequential_preLN__mha_block__moe_arch_mod__prompt'

def setup_inputs():
    _rng = _Rng(jax.random.key(int.from_bytes(__import__("os").urandom(4), "little")))
    _w = (lambda a: (lambda t: t.astype(jnp.bfloat16) if jnp.issubdtype(t.dtype, jnp.floating) else t)(jnp.asarray(a)))
    def _A_setup():
        B, S, D, H = 1, 2048, 512, 32
        return {
            "x": _w((lambda *s: _rng.normal(s) * 0.05)(B, S, D)),
            "wqkv": _w((lambda *s: _rng.normal(s) * 0.05)(D, 3 * D)),
            "wo": _w((lambda *s: _rng.normal(s) * 0.05)(D, D)),
        }
    _A_in = _A_setup()

    def _B_setup():
        B, S, D, F, C = 1, 2048, 512, 1792, 2
        return {
            "x": _w((lambda *s: _rng.normal(s) * 0.05)(B, S, D)),
            "w_r": _w((lambda *s: _rng.normal(s) * 0.05)(D)),
            "w_gate": _w((lambda *s: _rng.normal(s) * 0.05)(D, F)),
            "w_up": _w((lambda *s: _rng.normal(s) * 0.05)(D, F)),
            "w_down": _w((lambda *s: _rng.normal(s) * 0.05)(F, D)),
        }
    _B_in = _B_setup()

    return {
        "A_x": _A_in["x"],
        "A_wqkv": _A_in["wqkv"],
        "A_wo": _A_in["wo"],
        "B_x": _B_in["x"],
        "B_w_r": _B_in["w_r"],
        "B_w_gate": _B_in["w_gate"],
        "B_w_up": _B_in["w_up"],
        "B_w_down": _B_in["w_down"],
    }

def reference(A_x, A_wqkv, A_wo, B_x, B_w_r, B_w_gate, B_w_up, B_w_down):
    def _A_ref(x, wqkv, wo):
        B, S, D = x.shape
        H = 32
        Dh = D // H
        qkv = (lambda x, *d: x.transpose(*d))((x @ wqkv).reshape(B, S, 3, H, Dh), 2, 0, 3, 1, 4)
        q, k, v = qkv[0], qkv[1], qkv[2]
        scores = jnp.einsum("bhqd,bhkd->bhqk", q, k) * (Dh ** -0.5)
        p = _softmax(scores, axis=-1)
        o = jnp.einsum("bhqk,bhkd->bhqd", p, v)
        return (lambda x, *d: x.transpose(*d))(o, 0, 2, 1, 3).reshape(B, S, D) @ wo

    def _B_ref(x, w_r, w_gate, w_up, w_down):
        B, S, D = x.shape
        C = 2
        r = x @ w_r
        idx = jnp.argsort(-r, axis=-1)[:, :C]
        idx_e = jnp.repeat(idx.reshape(B, C, 1), D, axis=2)
        x_sel = jnp.take_along_axis(x, idx_e, axis=1)
        g = _silu(x_sel @ w_gate)
        u = x_sel @ w_up
        y = (g * u) @ w_down
        r_sel = _sigmoid(jnp.take_along_axis(r, idx, axis=1))
        y = y * r_sel.reshape(B, C, 1)
        b_off = (jnp.arange(B) * S).reshape(B, 1)
        flat_idx = (idx + b_off).reshape(B * C)
        zero = (x * 0.0).reshape(B * S, D)
        upd = _scatter_add(zero, flat_idx, y.reshape(B * C, D), axis=0)
        return x + upd.reshape(B, S, D)

    x = A_x
    h = x + _A_ref(_layernorm(x, axis=-1), A_wqkv, A_wo)
    h2 = h + _B_ref(_layernorm(h, axis=-1), B_w_r, B_w_gate, B_w_up, B_w_down)
    return h2
```

```python
import functools

import jax
import jax.numpy as jnp
import numpy as np
from jax import lax
from jax.experimental import pallas as pl
from jax.experimental.pallas import tpu as pltpu

bf16, f32, i32 = jnp.bfloat16, jnp.float32, jnp.int32

S, D, H, DH, F, CAP = 2048, 512, 32, 16, 1792, 2
BQ = 512
NQ = S // BQ
NT = S // 128
EPS = 1e-5
QSCALE = float(DH ** -0.5 * np.log2(np.e))
L_LO, L_HI = 2.0 ** -60, 2.0 ** 60
NN = (((1,), (0,)), ((), ()))
NT_DIMS = (((1,), (1,)), ((), ()))


def _rb(x):
    return x.astype(bf16).astype(f32)


def build(nvs=(1, 2, 1, 1), lagd=9, pc=512, ec=256, vshift=0, flags=None, skip=()):
    nvt = [nvs[j % len(nvs)] for j in range(NT)]
    vslabs = [(j, r) for j in range(NT) for r in range(7, 7 - nvt[j], -1)]
    vindex = {jr: n for n, jr in enumerate(vslabs)}
    nv = len(vslabs)

    def kernel(x_hbm, wqkv_hbm, wo_hbm, wr_ref, wg_hbm, wu_hbm, wd_hbm, out_hbm,
               x_v, wqkv_v, wo_v, wg_v, wu_v, wd_v, wt_v, k_s, q_s, v_s, kv_s,
               kb_a, kb_b, o_s, hn_s, sum_s, out_v, bad_s, junk_s, fix_v,
               sem_x, sem_w, sem_o, sem_f):
        npc = S // pc
        nec = S // ec

        def x_copy(c):
            rows = pl.ds(c * pc, pc)
            return pltpu.make_async_copy(x_hbm.at[rows], x_v.at[rows], sem_x.at[c])

        def wqkv_copy(n):
            cols = pl.ds(n * D, D)
            return pltpu.make_async_copy(wqkv_hbm.at[:, cols], wqkv_v.at[n], sem_w.at[n])

        late = [pltpu.make_async_copy(s, d, sem_w.at[3 + n]) for n, (s, d) in enumerate(
            [(wo_hbm, wo_v), (wg_hbm, wg_v), (wu_hbm, wu_v), (wd_hbm, wd_v)])]

        wqkv_copy(0).start()
        x_copy(0).start()
        wqkv_copy(2).start()
        wqkv_copy(1).start()
        for c in range(1, npc):
            x_copy(c).start()
        for cp in late:
            cp.start()

        wqkv_copy(0).wait()
        wt_v[0:D, :] = wqkv_v[0].T
        wqkv_copy(2).wait()
        wt_v[D:2 * D, :] = wqkv_v[2].T
        wqkv_copy(1).wait()

        for c in range(npc):
            x_copy(c).wait()
            xf = x_v[c * pc:(c + 1) * pc, :].astype(f32)
            mean = jnp.mean(xf, axis=-1, keepdims=True)
            xc = xf - mean
            var = jnp.mean(xc * xc, axis=-1, keepdims=True)
            den = _rb(jnp.sqrt(_rb(_rb(var) + float(np.asarray(EPS, ml_bf16)))))
            xn = (_rb(xf - _rb(mean)) / den).astype(bf16)
            qv = lax.dot_general(wt_v[...], xn, NT_DIMS, preferred_element_type=f32)
            cols = slice(c * pc, (c + 1) * pc)
            q_s[:, :, cols] = (qv[0:D] * QSCALE).reshape(H, DH, pc)
            v_s[:, :, cols] = qv[D:2 * D].reshape(H, DH, pc).astype(bf16)
            kk = lax.dot_general(xn, wqkv_v[1], NN, preferred_element_type=f32)
            kp = pltpu.bitcast(kk.astype(bf16), i32)
            for g in range(4):
                kg = kp[:, g * 128:(g + 1) * 128]
                for j in range(8):
                    k_s[8 * g + j, c * pc // 2:(c + 1) * pc // 2, :] = (
                        kg if j == 0 else pltpu.roll(kg, 128 - DH * j, 1))
                for (jt, r), n in vindex.items():
                    r0 = jt * 128 + 16 * r - c * pc
                    if 0 <= r0 < pc:
                        kv_s[g, n] = _rb(kk[r0:r0 + 16, g * 128:(g + 1) * 128])

        def kb_pieces(h, kb_ref):
            g = h // 8
            base = (h % 8) * DH
            for d in range(DH):
                idx = jnp.full((16, 128), d, i32) + base
                for n in range(nv):
                    kb_ref[n, d] = jnp.take_along_axis(kv_s[g, n], idx, axis=1)
                    yield

        for _ in kb_pieces(jnp.int32(0), kb_a):
            pass

        low = lax.broadcasted_iota(i32, (8, 128), 1) < DH
        bad_s[...] = jnp.zeros(bad_s.shape, f32)

        def attend(heads):
            tiles = [(u, qi, j) for u in range(len(heads)) for qi in range(NQ) for j in range(NT)]
            ms = [(t, r) for t, (_, _, j) in enumerate(tiles) for r in range(7 - nvt[j], -1, -1)]
            vs = [(t, r) for t, (_, _, j) in enumerate(tiles) for r in range(7, 7 - nvt[j], -1)]
            last = {t: n for n, (t, _) in enumerate(ms)}
            parts, lsum, acc = {}, {}, {}

            def absorb(t, r, s):
                key = tiles[t][:2]
                p = jnp.exp2(s)
                lsum[key] = p[0:8] if key not in lsum else lsum[key] + p[0:8]
                lsum[key] = lsum[key] + p[8:16]
                parts[t, r] = p

            def vpu_scores():
                for t, r in vs:
                    u, qi, j = tiles[t]
                    h, kb_ref = heads[u][:2]
                    a = [None] * 4
                    for d in range(DH):
                        kb = kb_ref[vindex[j, r], d]
                        for c in range(4):
                            c0 = qi * BQ + c * 128
                            term = kb * q_s[h, d:d + 1, c0:c0 + 128]
                            a[c] = term if a[c] is None else a[c] + term
                        if d == DH - 1:
                            absorb(t, r, jnp.concatenate(a, axis=1))
                        yield a[3]

            gen = vpu_scores()
            done = [0]

            def advance(target):
                a = None
                while done[0] < min(target, DH * len(vs)):
                    a = next(gen)
                    done[0] += 1
                return a

            def pv(t):
                u, qi, j = tiles[t]
                h = heads[u][0]
                advance(DH * sum(1 for tt, _ in vs if tt <= t))
                p = jnp.concatenate([parts.pop((t, r)) for r in range(8)], axis=0)
                o = lax.dot_general(v_s[h, :, j * 128:(j + 1) * 128], p, NN,
                                    preferred_element_type=f32)
                key = (u, qi)
                acc[key] = o if key not in acc else acc[key] + o
                if j == NT - 1:
                    l = jnp.sum(lsum[key], axis=0, keepdims=True)
                    a = acc[key]
                    o_s[h, :, qi * BQ:(qi + 1) * BQ] = a * (1.0 / l)
                    amax = jnp.maximum(jnp.abs(a[0:8]), jnp.abs(a[8:16]))
                    ok = (l >= L_LO) & (l <= L_HI) & (amax < np.inf)
                    bad_s[...] = jnp.where(ok, bad_s[...], 1.0)

            group = []

            def flush():
                if not group:
                    return
                u, qi, _ = tiles[group[0][0]]
                h = heads[u][0]
                kk = pltpu.bitcast(jnp.concatenate([e[2] for e in group], axis=0), bf16)[:, :DH]
                s = lax.dot_general(kk, q_s[h, :, qi * BQ:(qi + 1) * BQ], NN,
                                    preferred_element_type=f32)
                for m, (t, r, _) in enumerate(group):
                    absorb(t, r, s[16 * m:16 * m + 16])
                group.clear()

            nxt = slot = 0
            nslots = len(ms) + len(tiles)
            per_head = len(ms) // len(heads)
            kbg, kbd = None, 0
            for n, (t, r) in enumerate(ms):
                u, qi, j = tiles[t]
                if n % per_head == 0:
                    kbg, kbd = kb_pieces(heads[u][2], heads[u][3]), 0
                lo = 24
                want = min(DH * nv, max(0, (n % per_head - lo) * DH * nv // (per_head - 2 * lo)))
                while kbd < want:
                    next(kbg)
                    kbd += 1
                if group and tiles[group[0][0]][:2] != (u, qi):
                    flush()
                    pv(nxt)
                    nxt += 1
                    slot += 1
                ks = k_s[heads[u][0], j * 64 + 8 * r:j * 64 + 8 * r + 8, :]
                slot += 1
                a = advance((slot + vshift) * DH * len(vs) // nslots)
                if a is not None:
                    ks = jnp.where(low, ks, pltpu.bitcast(a[8:16], i32))
                group.append((t, r, ks))
                while nxt < len(tiles) and n >= last[nxt] + lagd:
                    flush()
                    pv(nxt)
                    nxt += 1
                    slot += 1
            flush()
            junk_s[...] = lsum[0, 0]
            while nxt < len(tiles):
                pv(nxt)
                nxt += 1

        def pair(i, carry):
            h0 = 2 * i
            attend([(h0, kb_a, h0 + 1, kb_b), (h0 + 1, kb_b, jnp.minimum(h0 + 2, H - 1), kb_a)])
            return carry

        if "att" not in skip:
            lax.fori_loop(0, H // 2, pair, 0)

        @pl.when(jnp.max(bad_s[...]) > 0.0)
        def _():
            def exact(n, carry):
                h = n // NQ
                c0 = pl.multiple_of((n % NQ) * BQ, BQ)
                kk = pltpu.bitcast(k_s[h], bf16)[:, :DH]
                s = lax.dot_general(kk, q_s[h, :, pl.ds(c0, BQ)], NN, preferred_element_type=f32)
                p = jnp.exp2(s - jnp.max(s, axis=0, keepdims=True))
                p = p * (1.0 / jnp.sum(p, axis=0, keepdims=True))
                o_s[h, :, pl.ds(c0, BQ)] = lax.dot_general(v_s[h], p, NN, preferred_element_type=f32)
                return carry

            lax.fori_loop(0, H * NQ, exact, 0)

        def out_copy(c):
            rows = pl.ds(c * ec, ec)
            return pltpu.make_async_copy(out_v.at[rows], out_hbm.at[rows], sem_o.at[c])

        late[0].wait()
        wr = wr_ref[...].astype(f32)
        sub = lax.broadcasted_iota(i32, (8, 1), 0)
        b1 = b2 = jnp.full((8, 1), -np.inf, f32)
        i1 = i2 = jnp.zeros((8, 1), i32)
        for c in range(nec):
            rows = slice(c * ec, (c + 1) * ec)
            ot = o_s[:, :, rows].reshape(D, ec)
            attn = lax.dot_general(ot.astype(bf16).T, wo_v[...], NN, preferred_element_type=f32)
            hf = x_v[rows, :].astype(f32) + attn
            hc = hf - jnp.mean(hf, axis=-1, keepdims=True)
            var = jnp.mean(hc * hc, axis=-1, keepdims=True)
            hn = hc * lax.rsqrt(var + EPS)
            tot = hf + hn
            hn_s[rows, :] = hn
            sum_s[rows, :] = tot
            out_v[rows, :] = tot.astype(bf16)
            out_copy(c).start()
            r = jnp.sum(hn * wr, axis=-1, keepdims=True)
            for m in range(ec // 8):
                rv = r[8 * m:8 * m + 8]
                iv = sub + (c * ec + 8 * m)
                gt1, gt2 = rv > b1, rv > b2
                b2 = jnp.where(gt1, b1, jnp.where(gt2, rv, b2))
                i2 = jnp.where(gt1, i1, jnp.where(gt2, iv, i2))
                b1 = jnp.where(gt1, rv, b1)
                i1 = jnp.where(gt1, iv, i1)

        big = 2 * S
        m1 = jnp.max(b1, axis=0, keepdims=True)
        t1 = jnp.min(jnp.where(b1 == m1, i1, big), axis=0, keepdims=True)
        won = i1 == t1
        cb, ci = jnp.where(won, b2, b1), jnp.where(won, i2, i1)
        m2 = jnp.max(cb, axis=0, keepdims=True)
        t2 = jnp.min(jnp.where(cb == m2, ci, big), axis=0, keepdims=True)
        tok1 = jnp.clip(t1[0, 0], 0, S - 1)
        tok2 = jnp.clip(t2[0, 0], 0, S - 1)

        row = lax.broadcasted_iota(i32, (16, D), 0)
        xs = jnp.where(row == 0, hn_s[pl.ds(tok1, 1), :],
                       jnp.where(row == 1, hn_s[pl.ds(tok2, 1), :], 0.0)).astype(bf16)
        late[1].wait()
        late[2].wait()
        late[3].wait()
        gate = lax.dot_general(xs, wg_v[...], NN, preferred_element_type=f32)
        up = lax.dot_general(xs, wu_v[...], NN, preferred_element_type=f32)
        act = (gate * jax.nn.sigmoid(gate) * up).astype(bf16)
        y = lax.dot_general(act, wd_v[...], NN, preferred_element_type=f32)
        y1 = y[0:1] * jax.nn.sigmoid(m1)
        y2 = y[1:2] * jax.nn.sigmoid(m2)

        g1 = pl.multiple_of((tok1 // 16) * 16, 16)
        g2 = pl.multiple_of((tok2 // 16) * 16, 16)
        for n, g in enumerate((g1, g2)):
            blk = sum_s[pl.ds(g, 16), :]
            blk = blk + jnp.where(row + g == tok1, y1, 0.0) + jnp.where(row + g == tok2, y2, 0.0)
            fix_v[n] = blk.astype(bf16)
        for c in range(nec):
            out_copy(c).wait()
        fix1 = pltpu.make_async_copy(fix_v.at[0], out_hbm.at[pl.ds(g1, 16)], sem_f.at[0])
        fix2 = pltpu.make_async_copy(fix_v.at[1], out_hbm.at[pl.ds(g2, 16)], sem_f.at[1])
        fix1.start()

        @pl.when(g1 != g2)
        def _():
            fix2.start()
            fix2.wait()

        fix1.wait()

    any_spec = pl.BlockSpec(memory_space=pl.ANY)
    scratch = [
        pltpu.VMEM((S, D), bf16),
        pltpu.VMEM((3, D, D), bf16),
        pltpu.VMEM((D, D), bf16),
        pltpu.VMEM((D, F), bf16),
        pltpu.VMEM((D, F), bf16),
        pltpu.VMEM((F, D), bf16),
        pltpu.VMEM((2 * D, D), bf16),
        pltpu.VMEM((H, S // 2, 128), i32),
        pltpu.VMEM((H, DH, S), f32),
        pltpu.VMEM((H, DH, S), bf16),
        pltpu.VMEM((4, nv, 16, 128), f32),
        pltpu.VMEM((nv, DH, 16, 128), f32),
        pltpu.VMEM((nv, DH, 16, 128), f32),
        pltpu.VMEM((H, DH, S), f32),
        pltpu.VMEM((S, D), f32),
        pltpu.VMEM((S, D), f32),
        pltpu.VMEM((S, D), bf16),
        pltpu.VMEM((8, BQ), f32),
        pltpu.VMEM((8, BQ), f32),
        pltpu.VMEM((2, 16, D), bf16),
        pltpu.SemaphoreType.DMA((S // pc,)),
        pltpu.SemaphoreType.DMA((7,)),
        pltpu.SemaphoreType.DMA((S // ec,)),
        pltpu.SemaphoreType.DMA((2,)),
    ]

    def fn(A_x, A_wqkv, A_wo, B_x, B_w_r, B_w_gate, B_w_up, B_w_down):
        out = pl.pallas_call(
            kernel,
            out_shape=jax.ShapeDtypeStruct((S, D), bf16),
            in_specs=[any_spec, any_spec, any_spec, pl.BlockSpec(memory_space=pltpu.VMEM),
                      any_spec, any_spec, any_spec],
            out_specs=any_spec,
            scratch_shapes=scratch,
            compiler_params=pltpu.CompilerParams(vmem_limit_bytes=110 * 1024 * 1024, flags=flags),
        )(A_x.reshape(S, D), A_wqkv, A_wo, B_w_r.reshape(1, D), B_w_gate, B_w_up, B_w_down)
        return out.reshape(1, S, D)

    return fn


ml_bf16 = jnp.bfloat16


@jax.jit
def pallas_sequential_preLN__mha_block__moe_arch_mod__prompt_kernel(
    A_x, A_wqkv, A_wo, B_x, B_w_r, B_w_gate, B_w_up, B_w_down
):
    return build()(A_x, A_wqkv, A_wo, B_x, B_w_r, B_w_gate, B_w_up, B_w_down)
```

```python
import jax
import jax.numpy as jnp
import numpy as np
from jax import lax
from jax.experimental import pallas as pl
from jax.experimental.pallas import tpu as pltpu

bf16, f32, i32 = jnp.bfloat16, jnp.float32, jnp.int32

S, D, H, DH, F = 2048, 512, 32, 16, 1792
BQ = 512
NQ = S // BQ
NT = S // 128
GROUP = 2
EPS = 1e-5
EPS_BF16 = float(np.asarray(EPS, bf16))
QSCALE = float(DH ** -0.5 * np.log2(np.e))
L_LO, L_HI, W_HI = 2.0 ** -60, 2.0 ** 60, 2.0 ** 48
SUM_PITCH = 9
X_CHUNKS = (2, 2, 12)
OUT_CHUNKS = (8, 6, 2)
NN = (((1,), (0,)), ((), ()))
NN_T = (((1,), (1,)), ((), ()))


def _dot(a, b, dims=NN):
    return lax.dot_general(a, b, dims, preferred_element_type=f32)


def _round_bf16(x):
    return x.astype(bf16).astype(f32)


def _pack(x):
    return pltpu.bitcast(x.astype(bf16), i32)


def _unpack(x):
    return pltpu.bitcast(x, bf16)


def _tile(t, size):
    return pl.ds(t * size if isinstance(t, int) else pl.multiple_of(t * size, size), size)


ALU_ROWS = (7, 4)
ALU_COUNT = (2, 1, 1, 2, 1, 1, 2, 1, 1, 2, 1, 2, 1, 1, 2, 1)
ALU_SLABS = {jr: n for n, jr in enumerate(
    (j, r) for j in range(NT) for r in ALU_ROWS[:ALU_COUNT[j] + (j == NT - 1)])}
NV = len(ALU_SLABS)
ALU_STEPS = 14
STAGE_STEPS = 88
PV_LAG = 9


def _kernel(x_hbm, wqkv_hbm, wo_hbm, wr_hbm, wg_hbm, wu_hbm, wd_hbm, out_hbm,
            x_v, wqkv_v, wo_v, wg_v, wu_v, wd_v, wt_p, wk_p, wo_p, xn_p, k_s, q_s, v_s,
            kv_s, kt_s, qt_s, p_a, head_a, head_b, order_s, p_b, o_s, l_s, il_s, ot_p,
            hn_s, h_s, out_v, fix_v, wr_v, sem_x, sem_w, sem_o, sem_f):

    def x_copy(c):
        rows = pl.ds(sum(X_CHUNKS[:c]) * 128, X_CHUNKS[c] * 128)
        return pltpu.make_async_copy(x_hbm.at[rows], x_v.at[rows], sem_x.at[c])

    def wqkv_copy(n):
        return pltpu.make_async_copy(
            wqkv_hbm.at[:, pl.ds(n * D, D)], wqkv_v.at[n], sem_w.at[n])

    def late_copies():
        pairs = ((wo_hbm, wo_v), (wr_hbm, wr_v.at[pl.ds(0, D)]),
                 (wg_hbm, wg_v), (wu_hbm, wu_v), (wd_hbm, wd_v))
        return [pltpu.make_async_copy(s, d, sem_w.at[3 + n]) for n, (s, d) in enumerate(pairs)]

    def out_copy(c):
        rows = pl.ds(sum(OUT_CHUNKS[:c]) * 128, OUT_CHUNKS[c] * 128)
        return pltpu.make_async_copy(out_v.at[rows], out_hbm.at[rows], sem_o.at[c])

    def norm1(t):
        for part in range(2):
            xf = x_v[_tile(2 * t + part, 64), :].astype(f32)
            mean = jnp.mean(xf, axis=-1, keepdims=True)
            xc = xf - mean
            var = jnp.mean(xc * xc, axis=-1, keepdims=True)
            den = _round_bf16(jnp.sqrt(_round_bf16(_round_bf16(var) + EPS_BF16)))
            xn_p[_tile(2 * t + part, 32), :] = _pack(_round_bf16(xf - _round_bf16(mean)) / den)

    def project_k(t):
        xn = _unpack(xn_p[_tile(t, 64), :])
        for g in range(4):
            lanes = _tile(g, 128)
            w = wqkv_v[1, :, lanes] if t == 0 else _unpack(wk_p[:, lanes])
            k_s[g, _tile(t, 64), :] = _pack(_dot(xn, w))

    def project_q(t):
        y = _dot(_unpack(wt_p[0]), _unpack(xn_p[_tile(t, 64), :]), NN_T)
        y = y.reshape(H, DH, 128) * QSCALE
        q_s[:, :, _tile(t, 128)] = y
        if t % 2 == 1:
            first = q_s[:, :, _tile(t - 1, 128)]
            b11, b21, b12, b22 = first[:, 0:8], first[:, 8:16], y[:, 0:8], y[:, 8:16]
            t1 = b12 - b11
            t2 = b22 - t1
            for m, term in enumerate((b21 - t2, t1, t2, b22 - b12)):
                qt_s[:, _tile(m, 8), _tile(t // 2, 128)] = term

    def query_term(h, m, d, pair):
        if m < 3:
            return q_s[h, pl.ds(8 * min(m, 1) + d, 1), _tile(2 * pair + m // 2, 128)]
        return qt_s[h, pl.ds(8 * (m - 3) + d, 1), _tile(pair, 128)]

    def project_v(t):
        y = _dot(_unpack(wt_p[1]), _unpack(xn_p[_tile(t, 64), :]), NN_T)
        v_s[:, :, _tile(t, 128)] = _pack(y).reshape(H, DH // 2, 128)

    def key_terms():
        for (j, r), n in ALU_SLABS.items():
            for g in range(4):
                keys = _unpack(k_s[g, _tile(8 * j + r, 8)]).astype(f32)
                for row in (n, n + 8) if n >= 16 else (n,):
                    kv_s[0, _tile(row, 8), _tile(g, 128)] = keys[0:8]
                    kv_s[1, _tile(row, 8), _tile(g, 128)] = keys[8:16]
        top = kv_s[0].T.reshape(H, DH, 256)
        bottom = kv_s[1].T.reshape(H, DH, 256)
        a11, a12, a21, a22 = top[:, 0:8], top[:, 8:16], bottom[:, 0:8], bottom[:, 8:16]
        s1 = a21 + a22
        s2 = s1 - a11
        terms = (a11, a12, a12 - s2, a22, s1, s2, a11 - a21)
        left = lax.broadcasted_iota(i32, (H, 8, 128), 2) < 64
        blocks = [term[:, :, 0:128] for term in terms] + [
            jnp.where(left, terms[2 * m][:, :, 128:], terms[min(2 * m + 1, 6)][:, :, 128:])
            for m in range(4)]
        for b, block in enumerate(blocks):
            kt_s[:, _tile(b // 2, 8), _tile(b % 2, 128)] = block

    def stage_head(h, dst, u):
        terms_ref, keys_ref = dst
        width = 8 * NV - 128
        for n in range(STAGE_STEPS):
            b, d = divmod(n, 8)
            row = kt_s[h, pl.ds(b // 2 * 8 + d, 1), _tile(b % 2, 128)]
            col = jnp.broadcast_to(row, (128, 128)).T
            if b < 7:
                terms_ref[u, n, 0:128] = col
            else:
                terms_ref[u, 16 * (b - 7) + d, 128:] = col[:width]
                if b < 10:
                    terms_ref[u, 16 * (b - 7) + 8 + d, 128:] = col[64:64 + width]
            if n % 5 == 0 and n // 5 < NT:
                rows = _tile(n // 5, 64)
                keys_ref[u, rows] = pltpu.roll(
                    k_s[h // 8, rows], (128 - DH * (h % 8)) % 128, 1)
            yield col[0:8]

    for copy in (x_copy(0), wqkv_copy(1), x_copy(1), wqkv_copy(0), x_copy(2),
                 wqkv_copy(2)):
        copy.start()
    for row in (NV, NV + 8):
        kv_s[:, pl.ds(8 * row, 8 * (24 - NV)), :] = jnp.zeros((2, 8 * (24 - NV), D), f32)
    p_b[...] = jnp.zeros(p_b.shape, i32)
    o_s[0, :, S - BQ:] = jnp.zeros((DH, BQ), f32)
    x_copy(0).wait()
    norm1(0)
    norm1(1)
    wqkv_copy(1).wait()
    project_k(0)
    wk_p[...] = _pack(wqkv_v[1])
    x_copy(1).wait()
    project_k(1)
    norm1(2)
    project_k(2)
    norm1(3)
    wqkv_copy(0).wait()
    project_k(3)
    wt_p[0] = _pack(wqkv_v[0].T)
    for t in range(4):
        project_q(t)
    x_copy(2).wait()
    for copy in late_copies():
        copy.start()
    norm1(4)
    for t in range(4, NT):
        project_k(t)
        if t < NT - 2:
            project_q(t)
        if t + 1 < NT:
            norm1(t + 1)
    wqkv_copy(2).wait()
    wt_p[1] = _pack(wqkv_v[2].T)
    wmax = jnp.max(jnp.abs(wqkv_v[2].astype(f32)).reshape(D // 8, 8, D), axis=0)
    project_q(NT - 2)
    key_terms()
    project_q(NT - 1)

    @pl.loop(0, GROUP)
    def _(u):
        staging = stage_head(u, head_a, u)
        for e in range(NT // GROUP):
            project_v(u * (NT // GROUP) + e)
            for _ in range(pl.cdiv(STAGE_STEPS, NT // GROUP - 1)):
                next(staging, None)

    lane = lax.broadcasted_iota(i32, (8, 128), 1)

    def last_tile(h, p_ref):
        o = _dot(_unpack(v_s[jnp.maximum(h - 1, 0), :, S - 128:]), _unpack(p_ref[...]))
        o_s[h, :, S - BQ:] = o_s[h, :, S - BQ:] + o
        return o

    def attend(h0, mine, following, p_in, p_out):
        tiles = [(u, qi, j) for u in range(GROUP) for qi in range(NQ) for j in range(NT)]
        final = len(tiles) - 1
        on_alu = [ALU_ROWS[:ALU_COUNT[j] + (t == final)] for t, (_, _, j) in enumerate(tiles)]
        mxu_work = [(t, r) for t in range(len(tiles)) for r in range(7, -1, -1)
                    if r not in on_alu[t]]
        alu_work = [(t, r) for t in range(len(tiles)) for r in on_alu[t]]
        last = {t: n for n, (t, _) in enumerate(mxu_work)}
        probs, sums, acc = {}, {}, {}

        def absorb(t, r, s):
            key = tiles[t][:2]
            p = jnp.exp2(s)
            sums[key] = p[0:8] if key not in sums else sums[key] + p[0:8]
            sums[key] = sums[key] + p[8:16]
            if t == final:
                p_out[_tile(r, 8), :] = _pack(p)
            else:
                probs[t, r] = p
            order_s[...] = sums[key]

        def alu_scores():
            for t, r in alu_work:
                u, qi, j = tiles[t]
                n = ALU_SLABS[j, r]

                def add(x, m, d):
                    keys = mine[0][u, 8 * m + d, _tile(n, 8)]
                    term = [keys * query_term(h0 + u, m, d, c) for c in (2 * qi, 2 * qi + 1)]
                    return term if x is None else both(x, term)

                def both(x, y):
                    return [x[0] + y[0], x[1] + y[1]]

                def pick(x, y, d):
                    return (x + y)[(d // 2 + 1) % 4]

                m1 = m5 = None
                for d in range(8):
                    m1, m5 = add(m1, 0, d), add(m5, 4, d)
                    if d % 2:
                        yield pick(m1, m5, d)
                c11 = u2 = m1
                for d in range(8):
                    c11, u2 = add(c11, 1, d), add(u2, 5, d)
                    if d % 2:
                        yield pick(c11, u2, d)
                u3, c12 = u2, both(u2, m5)
                for d in range(8):
                    u3, c12 = add(u3, 6, d), add(c12, 2, d)
                    if d % 2:
                        yield pick(c12, u3, d)
                c21, c22 = u3, both(u3, m5)
                for d in range(8):
                    c21 = add(c21, 3, d)
                    if d == 7:
                        absorb(t, r, jnp.concatenate([jnp.concatenate(
                            [x[0], y[0], x[1], y[1]], axis=1)
                            for x, y in ((c11, c12), (c21, c22))], axis=0))
                    if d % 4 == 3:
                        yield pick(c21, c21, d)

        scoring = alu_scores()
        done = [0]

        def advance(target):
            latest = None
            while done[0] < min(target, ALU_STEPS * len(alu_work)):
                latest = next(scoring)
                done[0] += 1
            return latest

        def weigh(t):
            u, qi, j = tiles[t]
            advance(ALU_STEPS * sum(len(rows) for rows in on_alu[:t + 1]))
            p = jnp.concatenate([probs.pop((t, r)) for r in range(8)], axis=0)
            o = _dot(_unpack(v_s[h0 + u, :, _tile(j, 128)]), p)
            acc[u, qi] = o if (u, qi) not in acc else acc[u, qi] + o
            if j == NT - 1 or t == final - 1:
                o_s[h0 + u + 1, :, _tile(qi, BQ)] = acc[u, qi]
            return o

        pending = []

        def score():
            if not pending:
                return
            u, qi, _ = tiles[pending[0][0]]
            keys = _unpack(jnp.concatenate([e[2] for e in pending], axis=0))[:, :DH]
            s = _dot(keys, q_s[h0 + u, :, _tile(qi, BQ)])
            for m, (t, r, _) in enumerate(pending):
                absorb(t, r, s[16 * m:16 * m + 16])
            pending.clear()

        weighed = slot = 0
        pace = ALU_STEPS * (len(alu_work) - 1) / (len(mxu_work) + len(tiles) + 1)
        due = {}
        for n, (t, r) in enumerate(mxu_work):
            u, qi, j = tiles[t]
            if n == 0 or tiles[mxu_work[n - 1][0]][0] != u:
                start, staged = n, 0
                staging = stage_head(jnp.minimum(h0 + u + GROUP, H - 1), following, u)
            if pending and tiles[pending[0][0]][:2] != (u, qi):
                score()
                weigh(weighed)
                weighed += 1
                slot += 1
            if n == 6:
                score()
                due[n + 9] = last_tile(h0, p_in)
                slot += 1
            slot += 1
            before = [advance(int(slot * pace))]
            while staged < min(STAGE_STEPS, (n - start) * STAGE_STEPS
                               // (len(mxu_work) // GROUP - 60)):
                col = next(staging)
                staged += 1
                if staged % 4 == 0:
                    before.append(col)
            if n in due:
                before += [due[n][8:16, c * 128:(c + 1) * 128] for c in (1, 3)]
            keys = mine[1][u, _tile(8 * j + r, 8), :]
            for m, x in enumerate(x for x in before if x is not None):
                keys = jnp.where(lane < DH * (m + 1), keys, pltpu.bitcast(x, i32))
            pending.append((t, r, keys))
            while weighed < final and n >= last[weighed] + PV_LAG:
                score()
                o = weigh(weighed)
                weighed += 1
                slot += 1
                if weighed <= 2:
                    due[n + 8] = o
        score()
        for t in range(weighed, final):
            weigh(t)
        advance(ALU_STEPS * len(alu_work))
        for (u, qi), l in sums.items():
            for c in range(4):
                l_s[4 * qi + c, pl.ds(SUM_PITCH * (h0 + u), 8), :] = l[:, c * 128:(c + 1) * 128]

    @pl.loop(0, H // (2 * GROUP))
    def _(i):
        h0 = 2 * GROUP * i
        pl.when(h0 < H)(lambda: attend(h0, head_a, head_b, p_b, p_a))
        pl.when(h0 + GROUP < H)(lambda: attend(h0 + GROUP, head_b, head_a, p_a, p_b))

    for copy in late_copies():
        copy.wait()
    last_tile(H, p_b)
    wo_p[...] = _pack(wo_v[...])

    unsafe = jnp.zeros((8, 128), f32)
    for c in range(4):
        unsafe = jnp.where(wmax[:, c * 128:(c + 1) * 128] <= W_HI, unsafe, 1.0)
    for t in range(NT):
        for g in range(4):
            l = l_s[t, pl.ds(8 * SUM_PITCH * g, 8, stride=SUM_PITCH), :]
            for r in range(1, 8):
                l = l + l_s[t, pl.ds(8 * SUM_PITCH * g + r, 8, stride=SUM_PITCH), :]
            unsafe = jnp.where((l >= L_LO) & (l <= L_HI), unsafe, 1.0)
            inv = pl.reciprocal(l, approx=True)
            il_s[_tile(g, 8), _tile(t, 128)] = inv + inv * (1.0 - l * inv)

    @pl.when(jnp.max(unsafe) > 0.0)
    def _():
        @pl.loop(0, H * NQ)
        def _(n):
            h = n // NQ
            cols = _tile(n % NQ, BQ)

            def accumulate(j, carry):
                m, l, o = carry
                keys = pltpu.roll(k_s[h // 8, _tile(j, 64)], (128 - DH * (h % 8)) % 128, 1)
                s = _dot(_unpack(keys)[:, :DH], q_s[h, :, cols])
                m_new = jnp.maximum(m, jnp.max(s, axis=0, keepdims=True))
                alpha = jnp.exp2(m - m_new)
                p = jnp.exp2(s - m_new)
                return (m_new, alpha * l + jnp.sum(p, axis=0, keepdims=True),
                        alpha * o + _dot(_unpack(v_s[h, :, _tile(j, 128)]), p * (1.0 / S)))

            _, l, o = lax.fori_loop(0, NT, accumulate, (
                jnp.full((1, BQ), float(np.finfo(np.float32).min), f32),
                jnp.zeros((1, BQ), f32), jnp.zeros((DH, BQ), f32)))
            o_s[h + 1, :, cols] = o * (S / l)

        il_s[...] = jnp.ones(il_s.shape, f32)

    wr = wr_v[0:D].astype(f32).reshape(1, D)
    sublane = lax.broadcasted_iota(i32, (8, 128), 0)

    def gather_heads(t):
        cols = _tile(t, 128)
        ot = jnp.concatenate(
            [o_s[h + 1, :, cols] * il_s[pl.ds(h, 1), cols] for h in range(H)], axis=0)
        ot_p[t % 2] = _pack(ot.astype(bf16).T)

    def project_out(t):
        o = _unpack(ot_p[t % 2])
        for g in range(4):
            cols = _tile(g, 128)
            h_s[_tile(t, 128), cols] = (x_v[_tile(t, 128), cols].astype(f32)
                                        + _dot(o, _unpack(wo_p[:, cols])))

    def norm2(t, first, second):
        hf = h_s[_tile(t, 128), :]
        hc = hf - jnp.mean(hf, axis=-1, keepdims=True)
        hn = hc * lax.rsqrt(jnp.mean(hc * hc, axis=-1, keepdims=True) + EPS)
        hn_s[_tile(t, 128), :] = hn
        out_v[_tile(t, 128), :] = (hf + hn).astype(bf16)
        r = jnp.broadcast_to(jnp.sum(hn * wr, axis=-1, keepdims=True), (128, 128))
        bits = pltpu.bitcast(jnp.clip(r, -3e38, 3e38), i32)
        for m in range(16):
            key = pltpu.bitcast((bits[8 * m:8 * m + 8] & -S)
                                | (S - 1 - t * 128 - 8 * m - sublane), f32)
            second = jnp.maximum(second, jnp.minimum(first, key))
            first = jnp.maximum(first, key)
        return first, second

    gather_heads(0)
    first = second = jnp.full((8, 128), -np.inf, f32)
    for t in range(NT + 1):
        if t + 1 < NT:
            gather_heads(t + 1)
        if t < NT:
            project_out(t)
        if t >= 1:
            first, second = norm2(t - 1, first, second)
        for c in range(len(OUT_CHUNKS)):
            if t == sum(OUT_CHUNKS[:c + 1]):
                out_copy(c).start()

    best = jnp.max(first, axis=0, keepdims=True)
    runner_up = jnp.max(jnp.where(first == best, second, first), axis=0, keepdims=True)

    def decode(key):
        bits = pltpu.bitcast(jnp.broadcast_to(key, (8, 128)), i32)
        return (S - 1 - (bits & (S - 1)))[0, 0], pltpu.bitcast(bits & -S, f32)[0:1, 0:1]

    tok1, r1 = decode(best)
    tok2, r2 = decode(runner_up)
    row = lax.broadcasted_iota(i32, (16, D), 0)
    xs = jnp.where(row == 0, hn_s[pl.ds(tok1, 1), :],
                   jnp.where(row == 1, hn_s[pl.ds(tok2, 1), :], 0.0)).astype(bf16)
    gate = _dot(xs, wg_v[...])
    act = (gate * jax.nn.sigmoid(gate) * _dot(xs, wu_v[...])).astype(bf16)
    y = _dot(act, wd_v[...])
    y1 = y[0:1] * jax.nn.sigmoid(r1)
    y2 = y[1:2] * jax.nn.sigmoid(r2)

    for n, tok in enumerate((tok1, tok2)):
        rows = _tile(tok // 16, 16)
        ids = row + tok // 16 * 16
        update = jnp.where(ids == tok1, y1, 0.0) + jnp.where(ids == tok2, y2, 0.0)
        fix_v[n] = (h_s[rows, :] + (hn_s[rows, :] + update)).astype(bf16)
    for c in range(len(OUT_CHUNKS)):
        out_copy(c).wait()

    def fix_copy(n, tok):
        return pltpu.make_async_copy(
            fix_v.at[n], out_hbm.at[_tile(tok // 16, 16)], sem_f.at[n])

    fix_copy(0, tok1).start()

    @pl.when(tok1 // 16 != tok2 // 16)
    def _():
        fix_copy(1, tok2).start()
        fix_copy(1, tok2).wait()

    fix_copy(0, tok1).wait()


_STAGED_HEADS = (pltpu.VMEM((GROUP, 56, 8 * NV, 128), f32),
                 pltpu.VMEM((GROUP, S // 2, 128), i32))
_SCRATCH = [
    pltpu.VMEM((S, D), bf16),
    pltpu.VMEM((3, D, D), bf16),
    pltpu.VMEM((D, D), bf16),
    pltpu.VMEM((D, F), bf16),
    pltpu.VMEM((D, F), bf16),
    pltpu.VMEM((F, D), bf16),
    pltpu.VMEM((2, D // 2, D), i32),
    pltpu.VMEM((D // 2, D), i32),
    pltpu.VMEM((D // 2, D), i32),
    pltpu.VMEM((S // 2, D), i32),
    pltpu.VMEM((4, S // 2, 128), i32),
    pltpu.VMEM((H, DH, S), f32),
    pltpu.VMEM((H, DH // 2, S), i32),
    pltpu.VMEM((2, 256, D), f32),
    pltpu.VMEM((H, 48, 256), f32),
    pltpu.VMEM((H, 32, S // 2), f32),
    pltpu.VMEM((64, BQ), i32),
    _STAGED_HEADS,
    _STAGED_HEADS,
    pltpu.VMEM((8, BQ), f32),
    pltpu.VMEM((64, BQ), i32),
    pltpu.VMEM((H + 1, DH, S), f32),
    pltpu.VMEM((NT, H * SUM_PITCH, 128), f32),
    pltpu.VMEM((H, S), f32),
    pltpu.VMEM((2, 64, D), i32),
    pltpu.VMEM((S, D), f32),
    pltpu.VMEM((S, D), f32),
    pltpu.VMEM((S, D), bf16),
    pltpu.VMEM((2, 16, D), bf16),
    pltpu.VMEM((16 * D,), bf16),
    pltpu.SemaphoreType.DMA((len(X_CHUNKS),)),
    pltpu.SemaphoreType.DMA((8,)),
    pltpu.SemaphoreType.DMA((len(OUT_CHUNKS),)),
    pltpu.SemaphoreType.DMA((2,)),
]


@jax.jit
def pallas_sequential_preLN__mha_block__moe_arch_mod__prompt_kernel(
    A_x, A_wqkv, A_wo, B_x, B_w_r, B_w_gate, B_w_up, B_w_down
):
    del B_x
    hbm = pl.BlockSpec(memory_space=pl.ANY)
    out = pl.pallas_call(
        _kernel,
        out_shape=jax.ShapeDtypeStruct((S, D), bf16),
        in_specs=[hbm] * 7,
        out_specs=hbm,
        scratch_shapes=_SCRATCH,
        compiler_params=pltpu.CompilerParams(vmem_limit_bytes=110 * 1024 * 1024),
    )(A_x.reshape(S, D), A_wqkv, A_wo, B_w_r, B_w_gate, B_w_up, B_w_down)
    return out.reshape(1, S, D)
```

```python
import jax
import jax.numpy as jnp
import numpy as np
from jax import lax
from jax.experimental import pallas as pl
from jax.experimental.pallas import tpu as pltpu

bf16, f32, i32 = jnp.bfloat16, jnp.float32, jnp.int32

S, D, H, DH, F = 2048, 512, 32, 16, 1792
BQ = 512
NQ = S // BQ
NT = S // 128
GROUP = 2
EPS = 1e-5
EPS_BF16 = float(np.asarray(EPS, bf16))
QSCALE = float(DH ** -0.5 * np.log2(np.e))
L_LO, L_HI, W_HI = 2.0 ** -80, 2.0 ** 100, 2.0 ** 16
SUM_PITCH = 9
X_CHUNKS = (2, 3, 11)
OUT_CHUNKS = (8, 6, 2)
NN = (((1,), (0,)), ((), ()))
NN_T = (((1,), (1,)), ((), ()))


def _dot(a, b, dims=NN):
    return lax.dot_general(a, b, dims, preferred_element_type=f32)


def _round_bf16(x):
    return x.astype(bf16).astype(f32)


def _pack(x):
    return pltpu.bitcast(x.astype(bf16), i32)


def _unpack(x):
    return pltpu.bitcast(x, bf16)


def _tile(t, size):
    return pl.ds(t * size if isinstance(t, int) else pl.multiple_of(t * size, size), size)


ALU_ROWS = (7, 4)
ALU_COUNT = (2, 1, 1, 2, 1, 1, 2, 1, 1, 2, 1, 2, 1, 1, 2, 1)
ALU_SLABS = {jr: n for n, jr in enumerate(
    (j, r) for j in range(NT) for r in ALU_ROWS[:ALU_COUNT[j] + (j == NT - 1)])}
NV = len(ALU_SLABS)
ALU_STEPS = 14
STAGE_STEPS = 88
PV_LAG = 9


def _kernel(x_hbm, wqkv_hbm, wo_hbm, wr_hbm, wg_hbm, wu_hbm, wd_hbm, out_hbm,
            x_v, wqkv_v, wo_v, wg_v, wu_v, wd_v, wt_p, wk_p, wo_p, xn_p, k_s, q_s, v_s,
            kv_s, kt_s, qt_s, p_a, head_a, head_b, order_s, p_b, o_s, l_s, il_s, ot_p,
            hn_s, h_s, out_v, fix_v, wr_v, sem_x, sem_w, sem_o, sem_f):

    def x_copy(c):
        rows = pl.ds(sum(X_CHUNKS[:c]) * 128, X_CHUNKS[c] * 128)
        return pltpu.make_async_copy(x_hbm.at[rows], x_v.at[rows], sem_x.at[c])

    def wqkv_copy(n):
        return pltpu.make_async_copy(
            wqkv_hbm.at[:, pl.ds(n * D, D)], wqkv_v.at[n], sem_w.at[n])

    def late_copies():
        pairs = ((wo_hbm, wo_v), (wr_hbm, wr_v.at[pl.ds(0, D)]),
                 (wg_hbm, wg_v), (wu_hbm, wu_v), (wd_hbm, wd_v))
        return [pltpu.make_async_copy(s, d, sem_w.at[3 + n]) for n, (s, d) in enumerate(pairs)]

    def out_copy(c):
        rows = pl.ds(sum(OUT_CHUNKS[:c]) * 128, OUT_CHUNKS[c] * 128)
        return pltpu.make_async_copy(out_v.at[rows], out_hbm.at[rows], sem_o.at[c])

    def norm1(t):
        for part in range(2):
            xf = x_v[_tile(2 * t + part, 64), :].astype(f32)
            mean = jnp.mean(xf, axis=-1, keepdims=True)
            xc = xf - mean
            var = jnp.mean(xc * xc, axis=-1, keepdims=True)
            den = _round_bf16(jnp.sqrt(_round_bf16(_round_bf16(var) + EPS_BF16)))
            xn_p[_tile(2 * t + part, 32), :] = _pack(_round_bf16(xf - _round_bf16(mean)) / den)

    def project_k(t):
        xn = _unpack(xn_p[_tile(t, 64), :])
        for g in range(4):
            lanes = _tile(g, 128)
            w = wqkv_v[1, :, lanes] if t == 0 else _unpack(wk_p[:, lanes])
            k_s[g, _tile(t, 64), :] = _pack(_dot(xn, w))

    def project_q(t):
        y = _dot(_unpack(wt_p[0]), _unpack(xn_p[_tile(t, 64), :]), NN_T)
        y = y.reshape(H, DH, 128) * QSCALE
        q_s[:, :, _tile(t, 128)] = y
        if t % 2 == 1:
            first = q_s[:, :, _tile(t - 1, 128)]
            b11, b21, b12, b22 = first[:, 0:8], first[:, 8:16], y[:, 0:8], y[:, 8:16]
            t1 = b12 - b11
            t2 = b22 - t1
            for m, term in enumerate((b21 - t2, t1, t2, b22 - b12)):
                qt_s[:, _tile(m, 8), _tile(t // 2, 128)] = term

    def query_term(h, m, d, pair):
        if m < 3:
            return q_s[h, pl.ds(8 * min(m, 1) + d, 1), _tile(2 * pair + m // 2, 128)]
        return qt_s[h, pl.ds(8 * (m - 3) + d, 1), _tile(pair, 128)]

    def project_v(t):
        y = _dot(_unpack(wt_p[1]), _unpack(xn_p[_tile(t, 64), :]), NN_T)
        v_s[:, :, _tile(t, 128)] = _pack(y).reshape(H, DH // 2, 128)

    def key_terms():
        for (j, r), n in ALU_SLABS.items():
            for g in range(4):
                keys = _unpack(k_s[g, _tile(8 * j + r, 8)]).astype(f32)
                for row in (n, n + 8) if n >= 16 else (n,):
                    kv_s[0, _tile(row, 8), _tile(g, 128)] = keys[0:8]
                    kv_s[1, _tile(row, 8), _tile(g, 128)] = keys[8:16]
        top = kv_s[0].T.reshape(H, DH, 256)
        bottom = kv_s[1].T.reshape(H, DH, 256)
        a11, a12, a21, a22 = top[:, 0:8], top[:, 8:16], bottom[:, 0:8], bottom[:, 8:16]
        s1 = a21 + a22
        s2 = s1 - a11
        terms = (a11, a12, a12 - s2, a22, s1, s2, a11 - a21)
        left = lax.broadcasted_iota(i32, (H, 8, 128), 2) < 64
        blocks = [term[:, :, 0:128] for term in terms] + [
            jnp.where(left, terms[2 * m][:, :, 128:], terms[min(2 * m + 1, 6)][:, :, 128:])
            for m in range(4)]
        for b, block in enumerate(blocks):
            kt_s[:, _tile(b // 2, 8), _tile(b % 2, 128)] = block

    def stage_head(h, dst, u):
        terms_ref, keys_ref = dst
        width = 8 * NV - 128
        for n in range(STAGE_STEPS):
            b, d = divmod(n, 8)
            row = kt_s[h, pl.ds(b // 2 * 8 + d, 1), _tile(b % 2, 128)]
            col = jnp.broadcast_to(row, (128, 128)).T
            if b < 7:
                terms_ref[u, n, 0:128] = col
            else:
                terms_ref[u, 16 * (b - 7) + d, 128:] = col[:width]
                if b < 10:
                    terms_ref[u, 16 * (b - 7) + 8 + d, 128:] = col[64:64 + width]
            if n % 5 == 0 and n // 5 < NT:
                rows = _tile(n // 5, 64)
                keys_ref[u, rows] = pltpu.roll(
                    k_s[h // 8, rows], (128 - DH * (h % 8)) % 128, 1)
            yield col[0:8]

    for copy in (x_copy(0), wqkv_copy(1), x_copy(1), wqkv_copy(0), x_copy(2),
                 wqkv_copy(2)):
        copy.start()
    for row in (NV, NV + 8):
        kv_s[:, pl.ds(8 * row, 8 * (24 - NV)), :] = jnp.zeros((2, 8 * (24 - NV), D), f32)
    p_b[...] = jnp.zeros(p_b.shape, i32)
    o_s[0, :, S - BQ:] = jnp.zeros((DH, BQ), f32)
    x_copy(0).wait()
    norm1(0)
    norm1(1)
    wqkv_copy(1).wait()
    project_k(0)
    wk_p[...] = _pack(wqkv_v[1])
    x_copy(1).wait()
    project_k(1)
    norm1(2)
    project_k(2)
    norm1(3)
    wqkv_copy(0).wait()
    project_k(3)
    wt_p[0] = _pack(wqkv_v[0].T)
    for t in range(4):
        project_q(t)
    norm1(4)
    x_copy(2).wait()
    for copy in late_copies():
        copy.start()
    for t in range(4, NT):
        project_k(t)
        if t < NT - 2:
            project_q(t)
        if t + 1 < NT:
            norm1(t + 1)
    wqkv_copy(2).wait()
    wt_p[1] = _pack(wqkv_v[2].T)
    wmax = jnp.max(jnp.abs(wqkv_v[2].astype(f32)).reshape(D // 8, 8, D), axis=0)
    project_q(NT - 2)
    key_terms()
    project_q(NT - 1)

    @pl.loop(0, GROUP)
    def _(u):
        staging = stage_head(u, head_a, u)
        for e in range(NT // GROUP):
            project_v(u * (NT // GROUP) + e)
            for _ in range(pl.cdiv(STAGE_STEPS, NT // GROUP - 1)):
                next(staging, None)

    lane = lax.broadcasted_iota(i32, (8, 128), 1)

    def last_tile(h, p_ref):
        o = _dot(_unpack(v_s[jnp.maximum(h - 1, 0), :, S - 128:]), _unpack(p_ref[...]))
        o_s[h, :, S - BQ:] = o_s[h, :, S - BQ:] + o
        return o

    def attend(h0, mine, following, p_in, p_out):
        tiles = [(u, qi, j) for u in range(GROUP) for qi in range(NQ) for j in range(NT)]
        final = len(tiles) - 1
        on_alu = [ALU_ROWS[:ALU_COUNT[j] + (t == final)] for t, (_, _, j) in enumerate(tiles)]
        mxu_work = [(t, r) for t in range(len(tiles)) for r in range(7, -1, -1)
                    if r not in on_alu[t]]
        alu_work = [(t, r) for t in range(len(tiles)) for r in on_alu[t]]
        last = {t: n for n, (t, _) in enumerate(mxu_work)}
        probs, sums, acc = {}, {}, {}

        def absorb(t, r, s):
            key = tiles[t][:2]
            p = jnp.exp2(s)
            sums[key] = p[0:8] if key not in sums else sums[key] + p[0:8]
            sums[key] = sums[key] + p[8:16]
            if t == final:
                p_out[_tile(r, 8), :] = _pack(p)
            else:
                probs[t, r] = p
            order_s[...] = sums[key]

        def alu_scores():
            for t, r in alu_work:
                u, qi, j = tiles[t]
                n = ALU_SLABS[j, r]

                def add(x, m, d):
                    keys = mine[0][u, 8 * m + d, _tile(n, 8)]
                    term = [keys * query_term(h0 + u, m, d, c) for c in (2 * qi, 2 * qi + 1)]
                    return term if x is None else both(x, term)

                def both(x, y):
                    return [x[0] + y[0], x[1] + y[1]]

                def pick(x, y, d, rot=1):
                    return (x + y)[(d // 2 + rot) % 4]

                m1 = m5 = None
                for d in range(8):
                    m1, m5 = add(m1, 0, d), add(m5, 4, d)
                    if d % 2:
                        yield pick(m1, m5, d)
                c11 = u2 = m1
                for d in range(8):
                    c11, u2 = add(c11, 1, d), add(u2, 5, d)
                    if d % 2:
                        yield pick(c11, u2, d, 0)
                u3, c12 = u2, both(u2, m5)
                for d in range(8):
                    u3, c12 = add(u3, 6, d), add(c12, 2, d)
                    if d % 2:
                        yield pick(c12, u3, d)
                c21, c22 = u3, both(u3, m5)
                for d in range(8):
                    c21 = add(c21, 3, d)
                    if d == 7:
                        absorb(t, r, jnp.concatenate([jnp.concatenate(
                            [x[0], y[0], x[1], y[1]], axis=1)
                            for x, y in ((c11, c12), (c21, c22))], axis=0))
                    if d % 4 == 3:
                        yield pick(c21, c21, d)

        scoring = alu_scores()
        done = [0]

        def advance(target):
            latest = None
            while done[0] < min(target, ALU_STEPS * len(alu_work)):
                latest = next(scoring)
                done[0] += 1
            return latest

        def weigh(t):
            u, qi, j = tiles[t]
            advance(ALU_STEPS * sum(len(rows) for rows in on_alu[:t + 1]))
            p = jnp.concatenate([probs.pop((t, r)) for r in range(8)], axis=0)
            o = _dot(_unpack(v_s[h0 + u, :, _tile(j, 128)]), p)
            acc[u, qi] = o if (u, qi) not in acc else acc[u, qi] + o
            if j == NT - 1 or t == final - 1:
                o_s[h0 + u + 1, :, _tile(qi, BQ)] = acc[u, qi]
            return o

        pending = []

        def score():
            if not pending:
                return
            u, qi, _ = tiles[pending[0][0]]
            keys = _unpack(jnp.concatenate([e[2] for e in pending], axis=0))[:, :DH]
            s = _dot(keys, q_s[h0 + u, :, _tile(qi, BQ)])
            for m, (t, r, _) in enumerate(pending):
                absorb(t, r, s[16 * m:16 * m + 16])
            pending.clear()

        weighed = slot = 0
        pace = ALU_STEPS * (len(alu_work) - 1) / (len(mxu_work) + len(tiles) + 1)
        due = {}
        for n, (t, r) in enumerate(mxu_work):
            u, qi, j = tiles[t]
            if n == 0 or tiles[mxu_work[n - 1][0]][0] != u:
                start, staged = n, 0
                staging = stage_head(jnp.minimum(h0 + u + GROUP, H - 1), following, u)
            if pending and tiles[pending[0][0]][:2] != (u, qi):
                score()
                weigh(weighed)
                weighed += 1
                slot += 1
            if n == 6:
                score()
                due[n + 9] = last_tile(h0, p_in)
                slot += 1
            slot += 1
            before = [advance(int(slot * pace))]
            while staged < min(STAGE_STEPS, (n - start) * STAGE_STEPS
                               // (len(mxu_work) // GROUP - 60)):
                col = next(staging)
                staged += 1
                if staged % 4 == 0:
                    before.append(col)
            if n in due:
                before += [due[n][8:16, c * 128:(c + 1) * 128] for c in (1, 3)]
            keys = mine[1][u, _tile(8 * j + r, 8), :]
            for m, x in enumerate(x for x in before if x is not None):
                keys = jnp.where(lane < DH * (m + 1), keys, pltpu.bitcast(x, i32))
            pending.append((t, r, keys))
            while weighed < final and n >= last[weighed] + PV_LAG:
                score()
                o = weigh(weighed)
                weighed += 1
                slot += 1
                if weighed <= 2:
                    due[n + 8] = o
        score()
        for t in range(weighed, final):
            weigh(t)
        advance(ALU_STEPS * len(alu_work))
        for (u, qi), l in sums.items():
            for c in range(4):
                l_s[4 * qi + c, pl.ds(SUM_PITCH * (h0 + u), 8), :] = l[:, c * 128:(c + 1) * 128]

    @pl.loop(0, H // (2 * GROUP))
    def _(i):
        h0 = 2 * GROUP * i
        pl.when(h0 < H)(lambda: attend(h0, head_a, head_b, p_b, p_a))
        pl.when(h0 + GROUP < H)(lambda: attend(h0 + GROUP, head_b, head_a, p_a, p_b))

    for copy in late_copies():
        copy.wait()
    last_tile(H, p_b)
    wo_p[...] = _pack(wo_v[...])

    huge_v = jnp.zeros((8, 128), f32)
    for c in range(4):
        huge_v = jnp.where(wmax[:, c * 128:(c + 1) * 128] <= W_HI, huge_v, 1.0)
    unsafe = [jnp.zeros((8, 128), f32)] * 4
    for t in range(NT):
        for g in range(4):
            l = l_s[t, pl.ds(8 * SUM_PITCH * g, 8, stride=SUM_PITCH), :]
            for r in range(1, 8):
                l = l + l_s[t, pl.ds(8 * SUM_PITCH * g + r, 8, stride=SUM_PITCH), :]
            unsafe[g] = jnp.where((l >= L_LO) & (l <= L_HI), unsafe[g], 1.0)
            inv = pl.reciprocal(l, approx=True)
            il_s[_tile(g, 8), _tile(t, 128)] = inv + inv * (1.0 - l * inv)

    def gather_heads(t):
        cols = _tile(t, 128)
        ot = jnp.concatenate(
            [o_s[h + 1, :, cols] * il_s[pl.ds(h, 1), cols] for h in range(H)], axis=0)
        ot_p[t % 2] = _pack(ot.astype(bf16).T)

    gather_heads(0)

    def redo(h, qi):
        cols = _tile(qi, BQ)

        def accumulate(j, carry):
            m, l, o = carry
            keys = pltpu.roll(k_s[h // 8, _tile(j, 64)], (128 - DH * (h % 8)) % 128, 1)
            s = _dot(_unpack(keys)[:, :DH], q_s[h, :, cols])
            m_new = jnp.maximum(m, jnp.max(s, axis=0, keepdims=True))
            alpha = jnp.exp2(m - m_new)
            p = jnp.exp2(s - m_new)
            return (m_new, alpha * l + jnp.sum(p, axis=0, keepdims=True),
                    alpha * o + _dot(_unpack(v_s[h, :, _tile(j, 128)]), p * (1.0 / S)))

        _, l, o = lax.fori_loop(0, NT, accumulate, (
            jnp.full((1, BQ), float(np.finfo(np.float32).min), f32),
            jnp.zeros((1, BQ), f32), jnp.zeros((DH, BQ), f32)))
        o_s[h + 1, :, cols] = o * (S / l)

    @pl.when(jnp.max(sum(unsafe, huge_v)) > 0.0)
    def _():
        for g in range(4):
            l_s[0, _tile(g, 8), :] = unsafe[g] + jnp.max(huge_v)

        @pl.loop(0, H)
        def _(h):
            @pl.when(jnp.max(l_s[0, pl.ds(h, 1), :]) > 0.0)
            def _():
                pl.loop(0, NQ)(lambda qi: redo(h, qi))
                rows = _tile(h // 8, 8)
                mine = lax.broadcasted_iota(i32, (8, S), 0) == h % 8
                il_s[rows, :] = jnp.where(mine, 1.0, il_s[rows, :])

        gather_heads(0)

    wr = wr_v[0:D].astype(f32).reshape(1, D)
    sublane = lax.broadcasted_iota(i32, (8, 128), 0)

    def project_out(t):
        o = _unpack(ot_p[t % 2])
        for g in range(4):
            cols = _tile(g, 128)
            h_s[_tile(t, 128), cols] = (x_v[_tile(t, 128), cols].astype(f32)
                                        + _dot(o, _unpack(wo_p[:, cols])))

    def norm2(t, first, second):
        hf = h_s[_tile(t, 128), :]
        hc = hf - jnp.mean(hf, axis=-1, keepdims=True)
        hn = hc * lax.rsqrt(jnp.mean(hc * hc, axis=-1, keepdims=True) + EPS)
        hn_s[_tile(t, 128), :] = hn
        out_v[_tile(t, 128), :] = (hf + hn).astype(bf16)
        r = jnp.broadcast_to(jnp.sum(hn * wr, axis=-1, keepdims=True), (128, 128))
        bits = pltpu.bitcast(jnp.clip(r, -3e38, 3e38), i32)
        for m in range(16):
            key = pltpu.bitcast((bits[8 * m:8 * m + 8] & -S)
                                | (S - 1 - t * 128 - 8 * m - sublane), f32)
            second = jnp.maximum(second, jnp.minimum(first, key))
            first = jnp.maximum(first, key)
        return first, second

    first = second = jnp.full((8, 128), -np.inf, f32)
    for t in range(NT + 1):
        if t + 1 < NT:
            gather_heads(t + 1)
        if t < NT:
            project_out(t)
        if t >= 1:
            first, second = norm2(t - 1, first, second)
        for c in range(len(OUT_CHUNKS)):
            if t == sum(OUT_CHUNKS[:c + 1]):
                out_copy(c).start()

    best = jnp.max(first, axis=0, keepdims=True)
    runner_up = jnp.max(jnp.where(first == best, second, first), axis=0, keepdims=True)

    def decode(key):
        bits = pltpu.bitcast(jnp.broadcast_to(key, (8, 128)), i32)
        return (S - 1 - (bits & (S - 1)))[0, 0], pltpu.bitcast(bits & -S, f32)[0:1, 0:1]

    tok1, r1 = decode(best)
    tok2, r2 = decode(runner_up)
    row = lax.broadcasted_iota(i32, (16, D), 0)
    xs = jnp.where(row == 0, hn_s[pl.ds(tok1, 1), :],
                   jnp.where(row == 1, hn_s[pl.ds(tok2, 1), :], 0.0)).astype(bf16)
    gate = _dot(xs, wg_v[...])
    act = (gate * jax.nn.sigmoid(gate) * _dot(xs, wu_v[...])).astype(bf16)
    y = _dot(act, wd_v[...])
    y1 = y[0:1] * jax.nn.sigmoid(r1)
    y2 = y[1:2] * jax.nn.sigmoid(r2)

    for n, tok in enumerate((tok1, tok2)):
        rows = _tile(tok // 16, 16)
        ids = row + tok // 16 * 16
        update = jnp.where(ids == tok1, y1, 0.0) + jnp.where(ids == tok2, y2, 0.0)
        fix_v[n] = (h_s[rows, :] + (hn_s[rows, :] + update)).astype(bf16)
    for c in range(len(OUT_CHUNKS)):
        out_copy(c).wait()

    def fix_copy(n, tok):
        return pltpu.make_async_copy(
            fix_v.at[n], out_hbm.at[_tile(tok // 16, 16)], sem_f.at[n])

    fix_copy(0, tok1).start()

    @pl.when(tok1 // 16 != tok2 // 16)
    def _():
        fix_copy(1, tok2).start()
        fix_copy(1, tok2).wait()

    fix_copy(0, tok1).wait()


_STAGED_HEADS = (pltpu.VMEM((GROUP, 56, 8 * NV, 128), f32),
                 pltpu.VMEM((GROUP, S // 2, 128), i32))
_SCRATCH = [
    pltpu.VMEM((S, D), bf16),
    pltpu.VMEM((3, D, D), bf16),
    pltpu.VMEM((D, D), bf16),
    pltpu.VMEM((D, F), bf16),
    pltpu.VMEM((D, F), bf16),
    pltpu.VMEM((F, D), bf16),
    pltpu.VMEM((2, D // 2, D), i32),
    pltpu.VMEM((D // 2, D), i32),
    pltpu.VMEM((D // 2, D), i32),
    pltpu.VMEM((S // 2, D), i32),
    pltpu.VMEM((4, S // 2, 128), i32),
    pltpu.VMEM((H, DH, S), f32),
    pltpu.VMEM((H, DH // 2, S), i32),
    pltpu.VMEM((2, 256, D), f32),
    pltpu.VMEM((H, 48, 256), f32),
    pltpu.VMEM((H, 32, S // 2), f32),
    pltpu.VMEM((64, BQ), i32),
    _STAGED_HEADS,
    _STAGED_HEADS,
    pltpu.VMEM((8, BQ), f32),
    pltpu.VMEM((64, BQ), i32),
    pltpu.VMEM((H + 1, DH, S), f32),
    pltpu.VMEM((NT, H * SUM_PITCH + 16, 128), f32),
    pltpu.VMEM((H, S), f32),
    pltpu.VMEM((2, 64, D), i32),
    pltpu.VMEM((S, D), f32),
    pltpu.VMEM((S, D), f32),
    pltpu.VMEM((S, D), bf16),
    pltpu.VMEM((2, 16, D), bf16),
    pltpu.VMEM((16 * D,), bf16),
    pltpu.SemaphoreType.DMA((len(X_CHUNKS),)),
    pltpu.SemaphoreType.DMA((8,)),
    pltpu.SemaphoreType.DMA((len(OUT_CHUNKS),)),
    pltpu.SemaphoreType.DMA((2,)),
]


@jax.jit
def pallas_sequential_preLN__mha_block__moe_arch_mod__prompt_kernel(
    A_x, A_wqkv, A_wo, B_x, B_w_r, B_w_gate, B_w_up, B_w_down
):
    del B_x
    hbm = pl.BlockSpec(memory_space=pl.ANY)
    out = pl.pallas_call(
        _kernel,
        out_shape=jax.ShapeDtypeStruct((S, D), bf16),
        in_specs=[hbm] * 7,
        out_specs=hbm,
        scratch_shapes=_SCRATCH,
        compiler_params=pltpu.CompilerParams(vmem_limit_bytes=110 * 1024 * 1024),
    )(A_x.reshape(S, D), A_wqkv, A_wo, B_w_r, B_w_gate, B_w_up, B_w_down)
    return out.reshape(1, S, D)
```

```python
import jax
import jax.numpy as jnp
import numpy as np
from jax import lax
from jax.experimental import pallas as pl
from jax.experimental.pallas import tpu as pltpu

bf16, f32, i32 = jnp.bfloat16, jnp.float32, jnp.int32

S, D, H, DH, F = 2048, 512, 32, 16, 1792
BQ = 512
NQ = S // BQ
NT = S // 128
GROUP = 2
EPS = 1e-5
EPS_BF16 = float(np.asarray(EPS, bf16))
QSCALE = float(DH ** -0.5 * np.log2(np.e))
L_LO, L_HI, W_HI = 2.0 ** -80, 2.0 ** 100, 2.0 ** 16
SUM_PITCH = 9
X_CHUNKS = (2, 3, 11)
OUT_CHUNKS = (8, 6, 2)
NN = (((1,), (0,)), ((), ()))
NN_T = (((1,), (1,)), ((), ()))


def _dot(a, b, dims=NN):
    return lax.dot_general(a, b, dims, preferred_element_type=f32)


def _round_bf16(x):
    return x.astype(bf16).astype(f32)


def _pack(x):
    return pltpu.bitcast(x.astype(bf16), i32)


def _unpack(x):
    return pltpu.bitcast(x, bf16)


def _tile(t, size):
    return pl.ds(t * size if isinstance(t, int) else pl.multiple_of(t * size, size), size)


ALU_ROWS = (7, 4)
ALU_COUNT = (2, 1, 1, 2, 1, 1, 2, 1, 1, 2, 1, 2, 1, 1, 2, 1)
ALU_SLABS = {jr: n for n, jr in enumerate(
    (j, r) for j in range(NT) for r in ALU_ROWS[:ALU_COUNT[j] + (j == NT - 1)])}
NV = len(ALU_SLABS)
ALU_STEPS = 14
STAGE_STEPS = 88
PV_LAG = 9


def _kernel(x_hbm, wqkv_hbm, wo_hbm, wr_hbm, wg_hbm, wu_hbm, wd_hbm, out_hbm,
            x_v, wqkv_v, wo_v, wg_v, wu_v, wd_v, wt_p, wk_p, wo_p, xn_p, k_s, q_s, v_s,
            kv_s, kt_s, qt_s, p_a, head_a, head_b, order_s, p_b, o_s, l_s, il_s, ot_p,
            hn_s, h_s, out_v, fix_v, wr_v, sem_x, sem_w, sem_o, sem_f):

    def x_copy(c):
        rows = pl.ds(sum(X_CHUNKS[:c]) * 128, X_CHUNKS[c] * 128)
        return pltpu.make_async_copy(x_hbm.at[rows], x_v.at[rows], sem_x.at[c])

    def wqkv_copy(n):
        return pltpu.make_async_copy(
            wqkv_hbm.at[:, pl.ds(n * D, D)], wqkv_v.at[n], sem_w.at[n])

    def late_copies(first, stop):
        pairs = ((wo_hbm, wo_v), (wr_hbm, wr_v.at[pl.ds(0, D)]),
                 (wg_hbm, wg_v), (wu_hbm, wu_v), (wd_hbm, wd_v))
        return [pltpu.make_async_copy(s, d, sem_w.at[3 + n])
                for n, (s, d) in enumerate(pairs) if first <= n < stop]

    def out_copy(c):
        rows = pl.ds(sum(OUT_CHUNKS[:c]) * 128, OUT_CHUNKS[c] * 128)
        return pltpu.make_async_copy(out_v.at[rows], out_hbm.at[rows], sem_o.at[c])

    def norm1(t):
        for part in range(2):
            xf = x_v[_tile(2 * t + part, 64), :].astype(f32)
            mean = jnp.mean(xf, axis=-1, keepdims=True)
            xc = xf - mean
            var = jnp.mean(xc * xc, axis=-1, keepdims=True)
            den = _round_bf16(jnp.sqrt(_round_bf16(_round_bf16(var) + EPS_BF16)))
            xn_p[_tile(2 * t + part, 32), :] = _pack(_round_bf16(xf - _round_bf16(mean)) / den)

    def project_k(t):
        xn = _unpack(xn_p[_tile(t, 64), :])
        for g in range(4):
            lanes = _tile(g, 128)
            w = wqkv_v[1, :, lanes] if t == 0 else _unpack(wk_p[:, lanes])
            k_s[g, _tile(t, 64), :] = _pack(_dot(xn, w))

    def project_q(t):
        y = _dot(_unpack(wt_p[0]), _unpack(xn_p[_tile(t, 64), :]), NN_T)
        y = y.reshape(H, DH, 128) * QSCALE
        q_s[:, :, _tile(t, 128)] = y
        if t % 2 == 1:
            first = q_s[:, :, _tile(t - 1, 128)]
            b11, b21, b12, b22 = first[:, 0:8], first[:, 8:16], y[:, 0:8], y[:, 8:16]
            t1 = b12 - b11
            t2 = b22 - t1
            for m, term in enumerate((b21 - t2, t1, t2, b22 - b12)):
                qt_s[:, _tile(m, 8), _tile(t // 2, 128)] = term

    def query_term(h, m, d, pair):
        if m < 3:
            return q_s[h, pl.ds(8 * min(m, 1) + d, 1), _tile(2 * pair + m // 2, 128)]
        return qt_s[h, pl.ds(8 * (m - 3) + d, 1), _tile(pair, 128)]

    def project_v(t):
        y = _dot(_unpack(wt_p[1]), _unpack(xn_p[_tile(t, 64), :]), NN_T)
        v_s[:, :, _tile(t, 128)] = _pack(y).reshape(H, DH // 2, 128)

    def key_terms():
        for (j, r), n in ALU_SLABS.items():
            for g in range(4):
                keys = _unpack(k_s[g, _tile(8 * j + r, 8)]).astype(f32)
                for row in (n, n + 8) if n >= 16 else (n,):
                    kv_s[0, _tile(row, 8), _tile(g, 128)] = keys[0:8]
                    kv_s[1, _tile(row, 8), _tile(g, 128)] = keys[8:16]
        top = kv_s[0].T.reshape(H, DH, 256)
        bottom = kv_s[1].T.reshape(H, DH, 256)
        a11, a12, a21, a22 = top[:, 0:8], top[:, 8:16], bottom[:, 0:8], bottom[:, 8:16]
        s1 = a21 + a22
        s2 = s1 - a11
        terms = (a11, a12, a12 - s2, a22, s1, s2, a11 - a21)
        left = lax.broadcasted_iota(i32, (H, 8, 128), 2) < 64
        blocks = [term[:, :, 0:128] for term in terms] + [
            jnp.where(left, terms[2 * m][:, :, 128:], terms[min(2 * m + 1, 6)][:, :, 128:])
            for m in range(4)]
        for b, block in enumerate(blocks):
            kt_s[:, _tile(b // 2, 8), _tile(b % 2, 128)] = block

    def stage_head(h, dst, u):
        terms_ref, keys_ref = dst
        width = 8 * NV - 128
        for n in range(STAGE_STEPS):
            b, d = divmod(n, 8)
            row = kt_s[h, pl.ds(b // 2 * 8 + d, 1), _tile(b % 2, 128)]
            col = jnp.broadcast_to(row, (128, 128)).T
            if b < 7:
                terms_ref[u, n, 0:128] = col
            else:
                terms_ref[u, 16 * (b - 7) + d, 128:] = col[:width]
                if b < 10:
                    terms_ref[u, 16 * (b - 7) + 8 + d, 128:] = col[64:64 + width]
            if n % 5 == 0 and n // 5 < NT:
                rows = _tile(n // 5, 64)
                keys_ref[u, rows] = pltpu.roll(
                    k_s[h // 8, rows], (128 - DH * (h % 8)) % 128, 1)
            yield col[0:8]

    for copy in (x_copy(0), wqkv_copy(1), x_copy(1), wqkv_copy(0), x_copy(2),
                 wqkv_copy(2)):
        copy.start()
    for row in (NV, NV + 8):
        kv_s[:, pl.ds(8 * row, 8 * (24 - NV)), :] = jnp.zeros((2, 8 * (24 - NV), D), f32)
    p_b[...] = jnp.zeros(p_b.shape, i32)
    o_s[0, :, S - BQ:] = jnp.zeros((DH, BQ), f32)
    x_copy(0).wait()
    norm1(0)
    norm1(1)
    wqkv_copy(1).wait()
    project_k(0)
    wk_p[...] = _pack(wqkv_v[1])
    x_copy(1).wait()
    project_k(1)
    norm1(2)
    project_k(2)
    norm1(3)
    wqkv_copy(0).wait()
    project_k(3)
    wt_p[0] = _pack(wqkv_v[0].T)
    for t in range(4):
        project_q(t)
    norm1(4)
    x_copy(2).wait()
    for copy in late_copies(0, 5):
        copy.start()
    for t in range(4, NT):
        project_k(t)
        if t < NT - 2:
            project_q(t)
        if t + 1 < NT:
            norm1(t + 1)
    wqkv_copy(2).wait()
    late_copies(0, 1)[0].wait()
    wt_p[1] = _pack(wqkv_v[2].T)
    wo_p[...] = _pack(wo_v[...])
    wmax = jnp.max(jnp.abs(wqkv_v[2].astype(f32)).reshape(D // 8, 8, D), axis=0)
    project_q(NT - 2)
    key_terms()
    project_q(NT - 1)

    @pl.loop(0, GROUP)
    def _(u):
        staging = stage_head(u, head_a, u)
        for e in range(NT // GROUP):
            project_v(u * (NT // GROUP) + e)
            for _ in range(pl.cdiv(STAGE_STEPS, NT // GROUP - 1)):
                next(staging, None)

    lane = lax.broadcasted_iota(i32, (8, 128), 1)

    def last_tile(h, p_ref):
        o = _dot(_unpack(v_s[jnp.maximum(h - 1, 0), :, S - 128:]), _unpack(p_ref[...]))
        o_s[h, :, S - BQ:] = o_s[h, :, S - BQ:] + o
        return o

    def attend(h0, mine, following, p_in, p_out):
        tiles = [(u, qi, j) for u in range(GROUP) for qi in range(NQ) for j in range(NT)]
        final = len(tiles) - 1
        on_alu = [ALU_ROWS[:ALU_COUNT[j] + (t == final)] for t, (_, _, j) in enumerate(tiles)]
        mxu_work = [(t, r) for t in range(len(tiles)) for r in range(7, -1, -1)
                    if r not in on_alu[t]]
        alu_work = [(t, r) for t in range(len(tiles)) for r in on_alu[t]]
        last = {t: n for n, (t, _) in enumerate(mxu_work)}
        probs, sums, acc = {}, {}, {}

        def absorb(t, r, s):
            key = tiles[t][:2]
            p = jnp.exp2(s)
            sums[key] = p[0:8] if key not in sums else sums[key] + p[0:8]
            sums[key] = sums[key] + p[8:16]
            if t == final:
                p_out[_tile(r, 8), :] = _pack(p)
            else:
                probs[t, r] = p
            order_s[...] = sums[key]

        def alu_scores():
            for t, r in alu_work:
                u, qi, j = tiles[t]
                n = ALU_SLABS[j, r]

                def add(x, m, d):
                    keys = mine[0][u, 8 * m + d, _tile(n, 8)]
                    term = [keys * query_term(h0 + u, m, d, c) for c in (2 * qi, 2 * qi + 1)]
                    return term if x is None else both(x, term)

                def both(x, y):
                    return [x[0] + y[0], x[1] + y[1]]

                def pick(x, y, d, rot=1):
                    return (x + y)[(d // 2 + rot) % 4]

                m1 = m5 = None
                for d in range(8):
                    m1, m5 = add(m1, 0, d), add(m5, 4, d)
                    if d % 2:
                        yield pick(m1, m5, d)
                c11 = u2 = m1
                for d in range(8):
                    c11, u2 = add(c11, 1, d), add(u2, 5, d)
                    if d % 2:
                        yield pick(c11, u2, d, 0)
                u3, c12 = u2, both(u2, m5)
                for d in range(8):
                    u3, c12 = add(u3, 6, d), add(c12, 2, d)
                    if d % 2:
                        yield pick(c12, u3, d)
                c21, c22 = u3, both(u3, m5)
                for d in range(8):
                    c21 = add(c21, 3, d)
                    if d == 7:
                        absorb(t, r, jnp.concatenate([jnp.concatenate(
                            [x[0], y[0], x[1], y[1]], axis=1)
                            for x, y in ((c11, c12), (c21, c22))], axis=0))
                    if d % 4 == 3:
                        yield pick(c21, c21, d)

        scoring = alu_scores()
        done = [0]

        def advance(target):
            latest = None
            while done[0] < min(target, ALU_STEPS * len(alu_work)):
                latest = next(scoring)
                done[0] += 1
            return latest

        def weigh(t):
            u, qi, j = tiles[t]
            advance(ALU_STEPS * sum(len(rows) for rows in on_alu[:t + 1]))
            p = jnp.concatenate([probs.pop((t, r)) for r in range(8)], axis=0)
            o = _dot(_unpack(v_s[h0 + u, :, _tile(j, 128)]), p)
            acc[u, qi] = o if (u, qi) not in acc else acc[u, qi] + o
            if j == NT - 1 or t == final - 1:
                o_s[h0 + u + 1, :, _tile(qi, BQ)] = acc[u, qi]
            return o

        pending = []

        def score():
            if not pending:
                return
            u, qi, _ = tiles[pending[0][0]]
            keys = _unpack(jnp.concatenate([e[2] for e in pending], axis=0))[:, :DH]
            s = _dot(keys, q_s[h0 + u, :, _tile(qi, BQ)])
            for m, (t, r, _) in enumerate(pending):
                absorb(t, r, s[16 * m:16 * m + 16])
            pending.clear()

        weighed = slot = 0
        pace = ALU_STEPS * (len(alu_work) - 1) / (len(mxu_work) + len(tiles) + 1)
        due = {}
        for n, (t, r) in enumerate(mxu_work):
            u, qi, j = tiles[t]
            if n == 0 or tiles[mxu_work[n - 1][0]][0] != u:
                start, staged = n, 0
                staging = stage_head(jnp.minimum(h0 + u + GROUP, H - 1), following, u)
            if pending and tiles[pending[0][0]][:2] != (u, qi):
                score()
                weigh(weighed)
                weighed += 1
                slot += 1
            if n == 6:
                score()
                due[n + 9] = last_tile(h0, p_in)
                slot += 1
            slot += 1
            before = [advance(int(slot * pace))]
            while staged < min(STAGE_STEPS, (n - start) * STAGE_STEPS
                               // (len(mxu_work) // GROUP - 60)):
                col = next(staging)
                staged += 1
                if staged % 4 == 0:
                    before.append(col)
            if n in due:
                before += [due[n][8:16, c * 128:(c + 1) * 128] for c in (1, 3)]
            keys = mine[1][u, _tile(8 * j + r, 8), :]
            for m, x in enumerate(x for x in before if x is not None):
                keys = jnp.where(lane < DH * (m + 1), keys, pltpu.bitcast(x, i32))
            pending.append((t, r, keys))
            while weighed < final and n >= last[weighed] + PV_LAG:
                score()
                o = weigh(weighed)
                weighed += 1
                slot += 1
                if weighed <= 2:
                    due[n + 8] = o
        score()
        for t in range(weighed, final):
            weigh(t)
        advance(ALU_STEPS * len(alu_work))
        for (u, qi), l in sums.items():
            for c in range(4):
                l_s[4 * qi + c, pl.ds(SUM_PITCH * (h0 + u), 8), :] = l[:, c * 128:(c + 1) * 128]

    @pl.loop(0, H // (2 * GROUP))
    def _(i):
        h0 = 2 * GROUP * i
        pl.when(h0 < H)(lambda: attend(h0, head_a, head_b, p_b, p_a))
        pl.when(h0 + GROUP < H)(lambda: attend(h0 + GROUP, head_b, head_a, p_a, p_b))

    for copy in late_copies(1, 5):
        copy.wait()
    last_tile(H, p_b)

    huge_v = jnp.zeros((8, 128), f32)
    for c in range(4):
        huge_v = jnp.where(wmax[:, c * 128:(c + 1) * 128] <= W_HI, huge_v, 1.0)
    unsafe = [jnp.zeros((8, 128), f32)] * 4
    for t in range(NT):
        for g in range(4):
            l = l_s[t, pl.ds(8 * SUM_PITCH * g, 8, stride=SUM_PITCH), :]
            for r in range(1, 8):
                l = l + l_s[t, pl.ds(8 * SUM_PITCH * g + r, 8, stride=SUM_PITCH), :]
            unsafe[g] = jnp.where((l >= L_LO) & (l <= L_HI), unsafe[g], 1.0)
            inv = pl.reciprocal(l, approx=True)
            il_s[_tile(g, 8), _tile(t, 128)] = inv + inv * (1.0 - l * inv)

    def gather_heads(t):
        cols = _tile(t, 128)
        ot = jnp.concatenate(
            [o_s[h + 1, :, cols] * il_s[pl.ds(h, 1), cols] for h in range(H)], axis=0)
        ot_p[t] = _pack(ot.astype(bf16).T)

    gather_heads(0)

    def redo(h, qi):
        cols = _tile(qi, BQ)

        def accumulate(j, carry):
            m, l, o = carry
            keys = pltpu.roll(k_s[h // 8, _tile(j, 64)], (128 - DH * (h % 8)) % 128, 1)
            s = _dot(_unpack(keys)[:, :DH], q_s[h, :, cols])
            m_new = jnp.maximum(m, jnp.max(s, axis=0, keepdims=True))
            alpha = jnp.exp2(m - m_new)
            p = jnp.exp2(s - m_new)
            return (m_new, alpha * l + jnp.sum(p, axis=0, keepdims=True),
                    alpha * o + _dot(_unpack(v_s[h, :, _tile(j, 128)]), p * (1.0 / S)))

        _, l, o = lax.fori_loop(0, NT, accumulate, (
            jnp.full((1, BQ), float(np.finfo(np.float32).min), f32),
            jnp.zeros((1, BQ), f32), jnp.zeros((DH, BQ), f32)))
        o_s[h + 1, :, cols] = o * (S / l)

    @pl.when(jnp.max(sum(unsafe, huge_v)) > 0.0)
    def _():
        for g in range(4):
            l_s[0, _tile(g, 8), :] = unsafe[g] + jnp.max(huge_v)

        @pl.loop(0, H)
        def _(h):
            @pl.when(jnp.max(l_s[0, pl.ds(h, 1), :]) > 0.0)
            def _():
                pl.loop(0, NQ)(lambda qi: redo(h, qi))
                rows = _tile(h // 8, 8)
                mine = lax.broadcasted_iota(i32, (8, S), 0) == h % 8
                il_s[rows, :] = jnp.where(mine, 1.0, il_s[rows, :])

        gather_heads(0)

    wr = wr_v[0:D].astype(f32).reshape(1, D)
    sublane = lax.broadcasted_iota(i32, (8, 128), 0)

    def project_out(t):
        o = _unpack(ot_p[t])
        for g in range(4):
            cols = _tile(g, 128)
            h_s[_tile(t, 128), cols] = (x_v[_tile(t, 128), cols].astype(f32)
                                        + _dot(o, _unpack(wo_p[:, cols])))

    def norm2(t, first, second):
        hf = h_s[_tile(t, 128), :]
        hc = hf - jnp.mean(hf, axis=-1, keepdims=True)
        hn = hc * lax.rsqrt(jnp.mean(hc * hc, axis=-1, keepdims=True) + EPS)
        hn_s[_tile(t, 128), :] = hn
        out_v[_tile(t, 128), :] = (hf + hn).astype(bf16)
        r = jnp.broadcast_to(jnp.sum(hn * wr, axis=-1, keepdims=True), (128, 128))
        bits = pltpu.bitcast(jnp.clip(r, -3e38, 3e38), i32)
        for m in range(16):
            key = pltpu.bitcast((bits[8 * m:8 * m + 8] & -S)
                                | (S - 1 - t * 128 - 8 * m - sublane), f32)
            second = jnp.maximum(second, jnp.minimum(first, key))
            first = jnp.maximum(first, key)
        return first, second

    first = second = jnp.full((8, 128), -np.inf, f32)
    for t in range(NT + 1):
        if t + 1 < NT:
            gather_heads(t + 1)
        if t < NT:
            project_out(t)
        if t >= 1:
            first, second = norm2(t - 1, first, second)
        for c in range(len(OUT_CHUNKS)):
            if t == sum(OUT_CHUNKS[:c + 1]):
                out_copy(c).start()

    best = jnp.max(first, axis=0, keepdims=True)
    runner_up = jnp.max(jnp.where(first == best, second, first), axis=0, keepdims=True)

    def decode(key):
        bits = pltpu.bitcast(jnp.broadcast_to(key, (8, 128)), i32)
        return (S - 1 - (bits & (S - 1)))[0, 0], pltpu.bitcast(bits & -S, f32)[0:1, 0:1]

    tok1, r1 = decode(best)
    tok2, r2 = decode(runner_up)
    row = lax.broadcasted_iota(i32, (16, D), 0)
    xs = jnp.where(row == 0, hn_s[pl.ds(tok1, 1), :],
                   jnp.where(row == 1, hn_s[pl.ds(tok2, 1), :], 0.0)).astype(bf16)
    gate = _dot(xs, wg_v[...])
    act = (gate * jax.nn.sigmoid(gate) * _dot(xs, wu_v[...])).astype(bf16)
    y = _dot(act, wd_v[...])
    y1 = y[0:1] * jax.nn.sigmoid(r1)
    y2 = y[1:2] * jax.nn.sigmoid(r2)

    for n, tok in enumerate((tok1, tok2)):
        rows = _tile(tok // 16, 16)
        ids = row + tok // 16 * 16
        update = jnp.where(ids == tok1, y1, 0.0) + jnp.where(ids == tok2, y2, 0.0)
        fix_v[n] = (h_s[rows, :] + (hn_s[rows, :] + update)).astype(bf16)
    for c in range(len(OUT_CHUNKS)):
        out_copy(c).wait()

    def fix_copy(n, tok):
        return pltpu.make_async_copy(
            fix_v.at[n], out_hbm.at[_tile(tok // 16, 16)], sem_f.at[n])

    fix_copy(0, tok1).start()

    @pl.when(tok1 // 16 != tok2 // 16)
    def _():
        fix_copy(1, tok2).start()
        fix_copy(1, tok2).wait()

    fix_copy(0, tok1).wait()


_STAGED_HEADS = (pltpu.VMEM((GROUP, 56, 8 * NV, 128), f32),
                 pltpu.VMEM((GROUP, S // 2, 128), i32))
_SCRATCH = [
    pltpu.VMEM((S, D), bf16),
    pltpu.VMEM((3, D, D), bf16),
    pltpu.VMEM((D, D), bf16),
    pltpu.VMEM((D, F), bf16),
    pltpu.VMEM((D, F), bf16),
    pltpu.VMEM((F, D), bf16),
    pltpu.VMEM((2, D // 2, D), i32),
    pltpu.VMEM((D // 2, D), i32),
    pltpu.VMEM((D // 2, D), i32),
    pltpu.VMEM((S // 2, D), i32),
    pltpu.VMEM((4, S // 2, 128), i32),
    pltpu.VMEM((H, DH, S), f32),
    pltpu.VMEM((H, DH // 2, S), i32),
    pltpu.VMEM((2, 256, D), f32),
    pltpu.VMEM((H, 48, 256), f32),
    pltpu.VMEM((H, 32, S // 2), f32),
    pltpu.VMEM((64, BQ), i32),
    _STAGED_HEADS,
    _STAGED_HEADS,
    pltpu.VMEM((8, BQ), f32),
    pltpu.VMEM((64, BQ), i32),
    pltpu.VMEM((H + 1, DH, S), f32),
    pltpu.VMEM((NT, H * SUM_PITCH + 16, 128), f32),
    pltpu.VMEM((H, S), f32),
    pltpu.VMEM((NT, 64, D), i32),
    pltpu.VMEM((S, D), f32),
    pltpu.VMEM((S, D), f32),
    pltpu.VMEM((S, D), bf16),
    pltpu.VMEM((2, 16, D), bf16),
    pltpu.VMEM((16 * D,), bf16),
    pltpu.SemaphoreType.DMA((len(X_CHUNKS),)),
    pltpu.SemaphoreType.DMA((8,)),
    pltpu.SemaphoreType.DMA((len(OUT_CHUNKS),)),
    pltpu.SemaphoreType.DMA((2,)),
]


@jax.jit
def pallas_sequential_preLN__mha_block__moe_arch_mod__prompt_kernel(
    A_x, A_wqkv, A_wo, B_x, B_w_r, B_w_gate, B_w_up, B_w_down
):
    del B_x
    hbm = pl.BlockSpec(memory_space=pl.ANY)
    out = pl.pallas_call(
        _kernel,
        out_shape=jax.ShapeDtypeStruct((S, D), bf16),
        in_specs=[hbm] * 7,
        out_specs=hbm,
        scratch_shapes=_SCRATCH,
        compiler_params=pltpu.CompilerParams(vmem_limit_bytes=110 * 1024 * 1024),
    )(A_x.reshape(S, D), A_wqkv, A_wo, B_w_r, B_w_gate, B_w_up, B_w_down)
    return out.reshape(1, S, D)
```
